```python
import os as _os
_os.environ.setdefault("JAX_PLATFORMS", "cpu")
import jax
import jax.numpy as jnp

def _softmax(x, axis=-1):
    return jax.nn.softmax(x, axis=axis)
def _gelu(x):
    return jax.nn.gelu(x, approximate=True)
def _silu(x):
    return jax.nn.silu(x)
def _sigmoid(x):
    return jax.nn.sigmoid(x)
def _layernorm(x, axis=-1, eps=1e-5):
    m = jnp.mean(x, axis=axis, keepdims=True)
    v = jnp.var(x, axis=axis, keepdims=True)
    return (x - m) / jnp.sqrt(v + eps)
def _scatter_add(tgt, idx, src, axis=0):
    return tgt.at[idx].add(src)
def _segment_sum(src, seg, n):
    return jax.ops.segment_sum(src, seg, n)
class _Rng:
    def __init__(self, key):
        self._k = key
    def _next(self):
        self._k, sub = jax.random.split(self._k)
        return sub
    def normal(self, shape):
        return jax.random.normal(self._next(), shape, dtype=jnp.bfloat16)
    def randint(self, lo, hi, shape):
        return jax.random.randint(self._next(), shape, lo, hi, dtype=jnp.int32)
    def uniform(self, shape, lo=0.0, hi=1.0):
        return jax.random.uniform(self._next(), shape, jnp.bfloat16, lo, hi)
    def permutation(self, n):
        return jax.random.permutation(self._next(), n)


kernel_name = 'interleave_layers__linear_kernel_hedgehog__ssm_conv_s4__prompt'

def setup_inputs():
    _rng = _Rng(jax.random.key(int.from_bytes(__import__("os").urandom(4), "little")))
    _w = (lambda a: (lambda t: t.astype(jnp.bfloat16) if jnp.issubdtype(t.dtype, jnp.floating) else t)(jnp.asarray(a)))
    def _A_setup():
        B, S, D, H = 1, 2048, 512, 32
        Dh = D // H
        return {
            "x": _w((lambda *s: _rng.normal(s) * 0.05)(B, S, D)),
            "wqkv": _w((lambda *s: _rng.normal(s) * 0.4)(D, 3 * D)),
            "w_phi": _w((lambda *s: _rng.normal(s) * 0.4)(H, Dh, Dh) * (Dh ** -0.5)),
            "wo": _w((lambda *s: _rng.normal(s) * 0.05)(D, D)),
        }
    _A_in = _A_setup()

    def _B_setup():
        B, L, D, N = 1, 2048, 512, 128
        A_re = -jnp.exp((lambda *s: _rng.normal(s) * 0.2)(D, N))
        A_im = jnp.pi * (lambda *s: _rng.normal(s) * 0.2)(D, N)
        B_re = (lambda *s: _rng.normal(s) * 0.2)(D, N)
        B_im = (lambda *s: _rng.normal(s) * 0.2)(D, N)
        C_re = (lambda *s: _rng.normal(s) * 0.2)(D, N)
        C_im = (lambda *s: _rng.normal(s) * 0.2)(D, N)
        log_dt = (lambda *s: _rng.normal(s) * 0.2)(D) * 0.5 - 4.0
        Dskip = (lambda *s: _rng.normal(s) * 0.2)(D)
        return {
            "u": _w((lambda *s: _rng.normal(s) * 0.05)(B, L, D)),
            "A_re": _w(A_re),
            "A_im": _w(A_im),
            "B_re": _w(B_re),
            "B_im": _w(B_im),
            "C_re": _w(C_re),
            "C_im": _w(C_im),
            "log_dt": _w(log_dt),
            "Dskip": _w(Dskip),
        }
    _B_in = _B_setup()

    return {
        "A_x": _A_in["x"],
        "A_wqkv": _A_in["wqkv"],
        "A_w_phi": _A_in["w_phi"],
        "A_wo": _A_in["wo"],
        "B_u": _B_in["u"],
        "B_A_re": _B_in["A_re"],
        "B_A_im": _B_in["A_im"],
        "B_B_re": _B_in["B_re"],
        "B_B_im": _B_in["B_im"],
        "B_C_re": _B_in["C_re"],
        "B_C_im": _B_in["C_im"],
        "B_log_dt": _B_in["log_dt"],
        "B_Dskip": _B_in["Dskip"],
    }

def reference(A_x, A_wqkv, A_w_phi, A_wo, B_u, B_A_re, B_A_im, B_B_re, B_B_im, B_C_re, B_C_im, B_log_dt, B_Dskip):
    def _A_ref(x, wqkv, w_phi, wo):
        B, S, D = x.shape
        H = 32; Dh = D // H
        qkv = (lambda x, *d: x.transpose(*d))((x @ wqkv).reshape(B, S, 3, H, Dh), 2, 0, 3, 1, 4)
        q, k, v = qkv[0], qkv[1], qkv[2]
        pq = jnp.einsum("bhsd,hdf->bhsf", q, w_phi)
        pk = jnp.einsum("bhsd,hdf->bhsf", k, w_phi)
        phi_q = jnp.concatenate([_softmax(pq, axis=-1), _softmax(-pq, axis=-1)], axis=-1)
        phi_k = jnp.concatenate([_softmax(pk, axis=-1), _softmax(-pk, axis=-1)], axis=-1)
        kv = jnp.einsum("bhsf,bhsd->bhfd", phi_k, v)
        z  = jnp.einsum("bhsf->bhf", phi_k)
        num = jnp.einsum("bhqf,bhfd->bhqd", phi_q, kv)
        den = jnp.einsum("bhqf,bhf->bhq", phi_q, z)[..., None] + 1e-6
        o = num / den
        return (lambda x, *d: x.transpose(*d))(o, 0, 2, 1, 3).reshape(B, S, D) @ wo

    def _B_ref(u, A_re, A_im, B_re, B_im, C_re, C_im, log_dt, Dskip):
        Bsz, L, D = u.shape
        dt = jnp.exp(log_dt)[:, None]
        A = A_re + 1j * A_im
        Bc = B_re + 1j * B_im
        Cc = C_re + 1j * C_im
        logdA = dt * A
        dB = dt * Bc
        l = (lambda x, dt: x.astype(dt))(jnp.arange(L), A_re.dtype)
        P = jnp.exp(logdA[:, :, None] * l[None, None, :])
        K = jnp.einsum("dn,dnl,dn->dl", Cc, P, dB).real
        L2 = 2 * L
        Kp = jnp.pad(K, ((0, 0), (0, L)))
        up = (lambda x, *d: x.transpose(*d))(u, 0, 2, 1)
        up = jnp.pad(up, ((0, 0), (0, 0), (0, L)))
        Kf = (lambda x, axes=(-2,-1): jnp.fft.rfft2(x.astype(jnp.float32), axes=axes))(Kp[:, None, :], axes=(-2, -1))
        Uf = (lambda x, axes=(-2,-1): jnp.fft.rfft2(x.astype(jnp.float32), axes=axes))(up[:, :, None, :], axes=(-2, -1))
        Yf = Uf * Kf[None, :, :, :]
        y = (lambda x, s, axes=(-2,-1): jnp.fft.irfft2(x, s=s, axes=axes).astype(jnp.bfloat16))(Yf, (1, L2), axes=(-2, -1))[:, :, 0, :L]
        y = (lambda x, *d: x.transpose(*d))(y, 0, 2, 1) + u * Dskip[None, None, :]
        return y

    x = A_x
    x = x + _A_ref(_layernorm(x, axis=-1), A_wqkv, A_w_phi, A_wo)
    x = x + _B_ref(_layernorm(x, axis=-1), B_A_re, B_A_im, B_B_re, B_B_im, B_C_re, B_C_im, B_log_dt, B_Dskip)
    x = x + _A_ref(_layernorm(x, axis=-1), A_wqkv, A_w_phi, A_wo)
    x = x + _B_ref(_layernorm(x, axis=-1), B_A_re, B_A_im, B_B_re, B_B_im, B_C_re, B_C_im, B_log_dt, B_Dskip)
    return x
```

```python
import functools
import numpy as np
import jax
import jax.numpy as jnp
from jax import lax
import jax.experimental.pallas as pl
import jax.experimental.pallas.tpu as pltpu
import ml_dtypes

S, D, H, DH, NS = 2048, 512, 32, 16, 128
F32, BF16 = jnp.float32, jnp.bfloat16
NT = (((1,), (1,)), ((), ()))
NN = (((1,), (0,)), ((), ()))


def _dft_consts():
    b = np.arange(128, dtype=np.float64)[:, None]
    k2 = np.arange(128, dtype=np.float64)[None, :]
    c = np.zeros((16, 128, 128), np.float64)
    s = np.zeros((16, 128, 128), np.float64)
    for k1 in range(16):
        ang = np.pi * b / 4096.0 - 2 * np.pi * b * (k1 + 16 * k2) / 2048.0
        c[k1] = np.cos(ang)
        s[k1] = np.sin(ang)
    return np.stack([c, s - c, c + s]).astype(ml_dtypes.bfloat16)


_DFT_M = _dft_consts()
KU = 32
BU = 4


def _cmulc(x, ang):
    c, s = float(np.cos(ang)), float(np.sin(ang))
    return (x[0] * c - x[1] * s, x[0] * s + x[1] * c)


def _cmul(x, y):
    return (x[0] * y[0] - x[1] * y[1], x[0] * y[1] + x[1] * y[0])


def _fft16_fwd(x):
    r2 = float(np.sqrt(0.5))
    c1, s1 = float(np.cos(np.pi / 8)), float(np.sin(np.pi / 8))
    Hh = [[None] * 4 for _ in range(4)]
    for a0 in range(4):
        x0, x1, x2, x3 = x[a0], x[4 + a0], x[8 + a0], x[12 + a0]
        m = x2 * r2
        t1 = (x1 * c1, x1 * s1)
        t3 = (x3 * s1, x3 * c1)
        p = x0 + m
        q = x0 - m
        u = (t1[0] + t3[0], t1[1] + t3[1])
        w = (t1[0] - t3[0], t1[1] - t3[1])
        Hh[a0][0] = (p + u[0], m + u[1])
        Hh[a0][2] = (p - u[0], m - u[1])
        Hh[a0][1] = (q + w[1], -m - w[0])
        Hh[a0][3] = (q - w[1], w[0] - m)
    G = [None] * 16
    for kp in range(4):
        t = [Hh[0][kp]] + [
            _cmulc(Hh[a0][kp], np.pi * a0 / 32 - 2 * np.pi * a0 * kp / 16) for a0 in range(1, 4)]
        s02 = (t[0][0] + t[2][0], t[0][1] + t[2][1])
        d02 = (t[0][0] - t[2][0], t[0][1] - t[2][1])
        s13 = (t[1][0] + t[3][0], t[1][1] + t[3][1])
        d13 = (t[1][0] - t[3][0], t[1][1] - t[3][1])
        G[kp] = (s02[0] + s13[0], s02[1] + s13[1])
        G[kp + 8] = (s02[0] - s13[0], s02[1] - s13[1])
        G[kp + 4] = (d02[0] + d13[1], d02[1] - d13[0])
        G[kp + 12] = (d02[0] - d13[1], d02[1] + d13[0])
    return G


def _fft16_inv(G):
    r2 = float(np.sqrt(0.5))
    c1, s1 = float(np.cos(np.pi / 8)), float(np.sin(np.pi / 8))
    J = [[None] * 4 for _ in range(4)]
    for kp in range(4):
        g0, g1, g2, g3 = G[kp], G[kp + 4], G[kp + 8], G[kp + 12]
        s02 = (g0[0] + g2[0], g0[1] + g2[1])
        d02 = (g0[0] - g2[0], g0[1] - g2[1])
        s13 = (g1[0] + g3[0], g1[1] + g3[1])
        d13 = (g1[0] - g3[0], g1[1] - g3[1])
        J[kp][0] = (s02[0] + s13[0], s02[1] + s13[1])
        J[kp][2] = (s02[0] - s13[0], s02[1] - s13[1])
        J[kp][1] = (d02[0] - d13[1], d02[1] + d13[0])
        J[kp][3] = (d02[0] + d13[1], d02[1] - d13[0])
    y = [None] * 16
    for a0 in range(4):
        t = [J[kp][a0] if (a0 == 0) else
             _cmulc(J[kp][a0], 2 * np.pi * a0 * kp / 16 - np.pi * a0 / 32) for kp in range(4)]
        s02 = (t[0][0] + t[2][0], t[0][1] + t[2][1])
        d02 = (t[0][0] - t[2][0], t[0][1] - t[2][1])
        s13 = (t[1][0] + t[3][0], t[1][1] + t[3][1])
        d13 = (t[1][0] - t[3][0], t[1][1] - t[3][1])
        z0r = s02[0] + s13[0]
        z2 = (s02[0] - s13[0], s02[1] - s13[1])
        z1 = (d02[0] - d13[1], d02[1] + d13[0])
        z3 = (d02[0] + d13[1], d02[1] - d13[0])
        y[a0] = z0r
        y[4 + a0] = z1[0] * c1 + z1[1] * s1
        y[8 + a0] = (z2[0] + z2[1]) * r2
        y[12 + a0] = z3[0] * s1 + z3[1] * c1
    return y


def _ln_t(x):
    m = jnp.mean(x, axis=0, keepdims=True)
    xc = x - m
    v = jnp.mean(xc * xc, axis=0, keepdims=True)
    return xc * lax.rsqrt(v + 1e-5)


def _phi(p):
    sl = [p[8 * f:8 * f + 8] for f in range(16)]
    mx = functools.reduce(jnp.maximum, sl)
    mn = functools.reduce(jnp.minimum, sl)
    ep = [jnp.exp(s - mx) for s in sl]
    en = [jnp.exp(mn - s) for s in sl]
    rp = 1.0 / functools.reduce(jnp.add, ep)
    rn = 1.0 / functools.reduce(jnp.add, en)
    out = jnp.concatenate([e * rp for e in ep] + [e * rn for e in en], axis=0)
    return out


TA = 256


def _kernel(x_hbm, wqkv_hbm, wphi_ref, wo_hbm, are_ref, aim_ref, bre_ref, bim_ref, cre_ref, cim_ref,
            ldt_ref, dsk_ref, dm_hbm, o_hbm,
            xt, un, xn, wt, wot, gb, gp, kh, tb, stp, kbuf, dcol, lhs_s, p0, p1r, pq_s, kvacc, zacc,
            xin_v, wqkv_v, wo_v, dm, ob0, ob1, sems):
    i32 = jnp.int32
    cp_x = pltpu.make_async_copy(x_hbm, xin_v, sems.at[0])
    cp_w = pltpu.make_async_copy(wqkv_hbm, wqkv_v, sems.at[1])
    cp_o = pltpu.make_async_copy(wo_hbm, wo_v, sems.at[2])
    cp_d = pltpu.make_async_copy(dm_hbm, dm, sems.at[3])
    cp_w.start()
    cp_o.start()
    cp_x.start()
    cp_d.start()

    with jax.named_scope("kgen_tab"):
        dt = jnp.exp(jnp.broadcast_to(ldt_ref[...].astype(F32), (128, 512)).T)
        dt = dt.astype(BF16).astype(F32)
        dcol[...] = jnp.broadcast_to(dsk_ref[...].astype(F32), (128, 512)).T
        ar = dt * are_ref[...].astype(F32)
        ai = dt * aim_ref[...].astype(F32)
        mag = jnp.exp(ar)
        lam = (mag * jnp.cos(ai), mag * jnp.sin(ai))
        db = (dt * bre_ref[...].astype(F32), dt * bim_ref[...].astype(F32))
        w = _cmul((cre_ref[...].astype(F32), cim_ref[...].astype(F32)), db)
        l2 = _cmul(lam, lam)
        l4 = _cmul(l2, l2)
        l8 = _cmul(l4, l4)
        l16 = _cmul(l8, l8)
        stp[0] = l16[0]
        stp[1] = l16[1]
        stp[6] = lam[0]
        stp[7] = lam[1]
        p = (jnp.ones_like(ar), jnp.zeros_like(ar))
        for j in range(8):
            tb[0, pl.ds(j, 512, stride=8), :] = p[0]
            tb[1, pl.ds(j, 512, stride=8), :] = p[1]
            if j < 7:
                p = _cmul(p, l2)
        l32 = _cmul(l16, l16)
        l64 = _cmul(l32, l32)
        l128 = _cmul(l64, l64)
        l256 = _cmul(l128, l128)
        stp[2] = l128[0]
        stp[3] = -l128[1]
        stp[4] = l64[0]
        stp[5] = -l64[1]
        stpc = (l256[0], -l256[1])
        p = (w[0], -w[1])
        for j in range(8):
            tb[2, pl.ds(j, 512, stride=8), :] = p[0]
            tb[3, pl.ds(j, 512, stride=8), :] = p[1]
            if j < 7:
                p = _cmul(p, stpc)

    with jax.named_scope("kgen_mm"):
        lane = lax.broadcasted_iota(i32, (16, 128), 1)
        lo = lane < 64
        pk = lambda x0, x1: pltpu.bitcast(pltpu.pack_elementwise([x0, x1], packed_dtype=BF16), BF16)

        def kg(i, _):
            for u in range(KU):
                Bs_r, Bs_i, As_r, As_i = [], [], [], []
                for e in range(2):
                    d = (i * KU + u) * 2 + e
                    d8 = pl.multiple_of(d * 8, 8)
                    bc = lambda k: jnp.broadcast_to(stp[k, pl.ds(d, 1), :], (8, 128))
                    s16 = (bc(0), bc(1))
                    ev = (tb[0, pl.ds(d8, 8), :], tb[1, pl.ds(d8, 8), :])
                    od = _cmul(ev, (bc(6), bc(7)))
                    for _k in range(4):
                        if _k:
                            ev = _cmul(ev, s16)
                            od = _cmul(od, s16)
                        Bs_r.append(pk(ev[0], od[0]))
                        Bs_i.append(pk(ev[1], od[1]))
                    a0 = (tb[2, pl.ds(d8, 8), :], tb[3, pl.ds(d8, 8), :])
                    a1 = _cmul(a0, (bc(2), bc(3)))
                    s64 = (bc(4), bc(5))
                    a2 = _cmul(a0, s64)
                    a3 = _cmul(a1, s64)
                    As_r += [pk(a0[0], a1[0]), pk(a2[0], a3[0])]
                    As_i += [pk(a0[1], a1[1]), pk(a2[1], a3[1])]
                cat = lambda z: jnp.concatenate(z, axis=0)
                lhs = jnp.concatenate([cat(As_r), cat(As_i)], axis=1)
                rhs = jnp.concatenate([cat(Bs_r), cat(Bs_i)], axis=1)
                out = lax.dot_general(lhs, rhs, NT, preferred_element_type=F32)
                t0 = jnp.where(lo, out[0:16], pltpu.roll(out[16:32], 64, 1))
                t1 = jnp.where(lo, pltpu.roll(out[32:48], 64, 1), out[48:64])
                d0 = (i * KU + u) * 2
                kbuf[pl.ds(d0, 16, stride=512), :] = t0
                kbuf[pl.ds(d0 + 1, 16, stride=512), :] = t1
            return 0
        lax.fori_loop(0, 256 // KU, kg, 0)

    def astage(src_fn, off):
        def body(rt, _):
            r0 = pl.multiple_of(rt * 16, 16)
            G = _fft16_fwd(src_fn(r0))
            for k1 in range(16):
                gb[k1, 0, pl.ds(off + r0, 16), :] = G[k1][0].astype(BF16)
                gb[k1, 1, pl.ds(off + r0, 16), :] = G[k1][1].astype(BF16)
                gb[k1, 2, pl.ds(off + r0, 16), :] = (G[k1][0] + G[k1][1]).astype(BF16)
            return 0
        lax.fori_loop(0, 32, body, 0)

    with jax.named_scope("kfft_a"):
        astage(lambda r0: [kbuf[pl.ds(512 * a + r0, 16), :] for a in range(16)], 0)

    with jax.named_scope("kfft_b"):
        cp_d.wait()

        def kb(i, _):
            for uu in range(BU):
                k1 = i * BU + uu
                t1 = lax.dot_general(gb[k1, 2], dm[0, k1], NN, preferred_element_type=F32)
                t2 = lax.dot_general(gb[k1, 0], dm[1, k1], NN, preferred_element_type=F32)
                t3 = lax.dot_general(gb[k1, 1], dm[2, k1], NN, preferred_element_type=F32)
                kh[k1, 0] = (t1 - t3) * (1.0 / 2048)
                kh[k1, 1] = (t1 + t2) * (1.0 / 2048)
            return 0
        lax.fori_loop(0, 16 // BU, kb, 0)

    with jax.named_scope("prep"):
        cp_w.wait()
        cp_o.wait()
        r = lax.broadcasted_iota(i32, (128, 128), 0)
        c = lax.broadcasted_iota(i32, (128, 128), 1)
        pv = jnp.where((r // 8 == c % 16) & (r % 8 == c // 16), 1.0, 0.0).astype(BF16)
        r16 = lax.broadcasted_iota(i32, (16, 128), 0)
        c16 = lax.broadcasted_iota(i32, (16, 128), 1)
        ex = jnp.where(r16 == c16 // 8, 1.0, 0.0).astype(BF16)
        hmask = (r // 16) == (c % 8)
        for g in range(4):
            wp = wphi_ref[128 * g:128 * g + 128, :]
            pt = jnp.where(hmask, lax.dot_general(wp, ex, NN, preferred_element_type=F32), 0.0)
            pg = pt.T.astype(BF16)
            for j in range(3):
                wg = wqkv_v[:, 512 * j + 128 * g:512 * j + 128 * g + 128]
                pm = pg if j < 2 else pv
                wt[512 * j + 128 * g:512 * j + 128 * g + 128, :] = lax.dot_general(
                    pm, wg, NT, preferred_element_type=F32).astype(BF16)
            tmp = lax.dot_general(pv, wo_v[128 * g:128 * g + 128, :], NN, preferred_element_type=F32)
            wot[:, 128 * g:128 * g + 128] = tmp.T.astype(BF16)
    with jax.named_scope("xin"):
        cp_x.wait()

        def xin(t, _):
            for u in range(2):
                t0 = pl.multiple_of((2 * t + u) * 128, 128)
                xv = xin_v[pl.ds(t0, 128), :].astype(F32).T
                xt[:, pl.ds(t0, 128)] = xv
                xn[:, pl.ds(t0, 128)] = _ln_t(xv).astype(BF16)
            return 0
        lax.fori_loop(0, 8, xin, 0)

    def attention(first):
        if not first:
            with jax.named_scope("a_ln"):
                def lnb(t, _):
                    for u in range(4):
                        t0 = pl.multiple_of((4 * t + u) * 128, 128)
                        xn[:, pl.ds(t0, 128)] = _ln_t(xt[:, pl.ds(t0, 128)]).astype(BF16)
                    return 0
                lax.fori_loop(0, 4, lnb, 0)
        with jax.named_scope("a_kv"):
            NTL = S // TA

            def qkv(t, pref):
                t0 = pl.multiple_of(t * TA, TA)
                pref[...] = lax.dot_general(wt[...], xn[:, pl.ds(t0, TA)], NN, preferred_element_type=F32)

            def soft(t, pref):
                t0 = pl.multiple_of(t * TA, TA)
                for g in range(4):
                    pq_s[256 * g:256 * g + 256, pl.ds(t0, TA)] = _phi(pref[128 * g:128 * g + 128, :]).astype(BF16)
                    phf = _phi(pref[512 + 128 * g:512 + 128 * g + 128, :])
                    v = pref[1024 + 128 * g:1024 + 128 * g + 128, :].astype(BF16)
                    kvacc[g] += lax.dot_general(phf.astype(BF16), v, NT, preferred_element_type=F32)
                    z = zacc[g]
                    for j in range(TA // 128):
                        z = z + phf[:, 128 * j:128 * j + 128]
                    zacc[g] = z
            kvacc[...] = jnp.zeros_like(kvacc)
            zacc[...] = jnp.zeros_like(zacc)
            qkv(0, p0)

            def p1(i, _):
                qkv(2 * i + 1, p1r)
                soft(2 * i, p0)
                qkv(2 * i + 2, p0)
                soft(2 * i + 1, p1r)
                return 0
            lax.fori_loop(0, NTL // 2 - 1, p1, 0)
            qkv(NTL - 1, p1r)
            soft(NTL - 2, p0)
            soft(NTL - 1, p1r)
            rr = lax.broadcasted_iota(i32, (128, 256), 0)
            cc = lax.broadcasted_iota(i32, (128, 256), 1)
            m1 = (rr % 8) == (cc % 8)
            r8 = lax.broadcasted_iota(i32, (16, 256), 0)
            c8 = lax.broadcasted_iota(i32, (16, 256), 1)
            m2 = r8 == (c8 % 8)
            for g in range(4):
                lhs_s[g, 0:128, :] = jnp.where(m1, kvacc[g].T, 0.0).astype(BF16)
                zrow = jnp.sum(zacc[g].T, axis=0, keepdims=True)
                lhs_s[g, 128:144, :] = jnp.where(m2, jnp.broadcast_to(zrow, (16, 256)), 0.0).astype(BF16)
        with jax.named_scope("a_q"):
            NTL = S // TA

            def sx(t, oref):
                t0 = pl.multiple_of(t * TA, TA)
                for g in range(4):
                    ph = pq_s[256 * g:256 * g + 256, pl.ds(t0, TA)]
                    nd = lax.dot_general(lhs_s[g], ph, NN, preferred_element_type=F32)
                    rden = 1.0 / (nd[128:136] + 1e-6)
                    oref[128 * g:128 * g + 128, :] = jnp.concatenate(
                        [nd[8 * dd:8 * dd + 8] * rden for dd in range(16)], axis=0).astype(BF16)

            def sy(t, oref):
                t0 = pl.multiple_of(t * TA, TA)
                acc = xt[:, pl.ds(t0, TA)] + lax.dot_general(wot[...], oref[...], NN, preferred_element_type=F32)
                u = _ln_t(acc)
                un[:, pl.ds(t0, TA)] = u
                dcv = dcol[...]
                xt[:, pl.ds(t0, TA)] = acc + u * jnp.concatenate([dcv] * (TA // 128), axis=1)
            sx(0, ob0)

            def p2(i, _):
                sx(2 * i + 1, ob1)
                sy(2 * i, ob0)
                sx(2 * i + 2, ob0)
                sy(2 * i + 1, ob1)
                return 0
            lax.fori_loop(0, NTL // 2 - 1, p2, 0)
            sx(NTL - 1, ob1)
            sy(NTL - 2, ob0)
            sy(NTL - 1, ob1)

    def conv(first):
        with jax.named_scope("b_a"):
            astage(lambda r0: [un[pl.ds(r0, 16), 128 * a:128 * a + 128] for a in range(16)], 0)
        with jax.named_scope("b_b"):
            def bb(i, _):
                for uu in range(BU):
                    k1 = i * BU + uu
                    m0, m1, m2 = dm[0, k1], dm[1, k1], dm[2, k1]
                    t1 = lax.dot_general(gb[k1, 2], m0, NN, preferred_element_type=F32)
                    t2 = lax.dot_general(gb[k1, 0], m1, NN, preferred_element_type=F32)
                    t3 = lax.dot_general(gb[k1, 1], m2, NN, preferred_element_type=F32)
                    xr, xi = t1 - t3, t1 + t2
                    kr, ki = kh[k1, 0], kh[k1, 1]
                    yr = xr * kr - xi * ki
                    yi = xr * ki + xi * kr
                    t1 = lax.dot_general((yr + yi).astype(BF16), m0, NT, preferred_element_type=F32)
                    t2 = lax.dot_general(yr.astype(BF16), m2, NT, preferred_element_type=F32)
                    t3 = lax.dot_general(yi.astype(BF16), m1, NT, preferred_element_type=F32)
                    gp[k1, 0] = t1 + t3
                    gp[k1, 1] = t1 - t2
                return 0
            lax.fori_loop(0, 16 // BU, bb, 0)
        with jax.named_scope("b_i"):
            def body(rt, _):
                r0 = pl.multiple_of(rt * 8, 8)
                G = [(gp[k1, 0, pl.ds(r0, 8), :], gp[k1, 1, pl.ds(r0, 8), :]) for k1 in range(16)]
                y = _fft16_inv(G)
                for a in range(16):
                    xt[pl.ds(r0, 8), 128 * a:128 * a + 128] = xt[pl.ds(r0, 8), 128 * a:128 * a + 128] + y[a]
                return 0
            lax.fori_loop(0, 64, body, 0)

    attention(True)
    conv(True)
    attention(False)
    conv(False)
    with jax.named_scope("xout"):
        def ocopy(t):
            return pltpu.make_async_copy(xin_v.at[pl.ds(t * 128, 128), :], o_hbm.at[pl.ds(t * 128, 128), :],
                                         sems.at[4])
        for t in range(16):
            xin_v[t * 128:t * 128 + 128, :] = xt[:, t * 128:t * 128 + 128].T.astype(BF16)
            ocopy(t).start()
        for t in range(16):
            ocopy(t).wait()


@jax.jit
def pallas_interleave_layers__linear_kernel_hedgehog__ssm_conv_s4__prompt_kernel(
    A_x, A_wqkv, A_w_phi, A_wo, B_u, B_A_re, B_A_im, B_B_re, B_B_im, B_C_re, B_C_im, B_log_dt, B_Dskip,
):
    del B_u
    vm = pl.BlockSpec(memory_space=pltpu.VMEM)
    hb = pl.BlockSpec(memory_space=pl.ANY)
    out = pl.pallas_call(
        _kernel,
        out_shape=jax.ShapeDtypeStruct((S, D), BF16),
        in_specs=[hb, hb, vm, hb, vm, vm, vm, vm, vm, vm, vm, vm, hb],
        out_specs=hb,
        scratch_shapes=[
            pltpu.VMEM((D, S), F32),
            pltpu.VMEM((D, S), F32),
            pltpu.VMEM((D, S), BF16),
            pltpu.VMEM((3 * D, D), BF16),
            pltpu.VMEM((D, D), BF16),
            pltpu.VMEM((16, 3, D, 128), BF16),
            pltpu.VMEM((16, 2, D, 128), F32),
            pltpu.VMEM((16, 2, D, 128), F32),
            pltpu.VMEM((4, D * 8, 128), F32),
            pltpu.VMEM((8, D, 128), F32),
            pltpu.VMEM((16 * D, 128), F32),
            pltpu.VMEM((D, 128), F32),
            pltpu.VMEM((4, 144, 256), BF16),
            pltpu.VMEM((3 * D, TA), F32),
            pltpu.VMEM((3 * D, TA), F32),
            pltpu.VMEM((2 * D, S), BF16),
            pltpu.VMEM((4, 256, 128), F32),
            pltpu.VMEM((4, 256, 128), F32),
            pltpu.VMEM((S, D), BF16),
            pltpu.VMEM((D, 3 * D), BF16),
            pltpu.VMEM((D, D), BF16),
            pltpu.VMEM((3, 16, 128, 128), BF16),
            pltpu.VMEM((D, TA), BF16),
            pltpu.VMEM((D, TA), BF16),
            pltpu.SemaphoreType.DMA((5,)),
        ],
        compiler_params=pltpu.CompilerParams(vmem_limit_bytes=120 * 1024 * 1024),
    )(A_x.reshape(S, D), A_wqkv, A_w_phi.reshape(H * DH, DH), A_wo,
      B_A_re, B_A_im, B_B_re, B_B_im, B_C_re, B_C_im,
      B_log_dt.reshape(1, D), B_Dskip.reshape(1, D), jnp.asarray(_DFT_M))
    return out.reshape(1, S, D)
```

```python
import functools
import numpy as np
import jax
import jax.numpy as jnp
from jax import lax
import jax.experimental.pallas as pl
import jax.experimental.pallas.tpu as pltpu
import ml_dtypes

S, D, H, DH, NS = 2048, 512, 32, 16, 128
F32, BF16 = jnp.float32, jnp.bfloat16
NT = (((1,), (1,)), ((), ()))
NN = (((1,), (0,)), ((), ()))


def _dft_consts():
    b = np.arange(128, dtype=np.float64)[:, None]
    k2 = np.arange(128, dtype=np.float64)[None, :]
    c = np.zeros((16, 128, 128), np.float64)
    s = np.zeros((16, 128, 128), np.float64)
    for k1 in range(16):
        ang = np.pi * b / 4096.0 - 2 * np.pi * b * (k1 + 16 * k2) / 2048.0
        c[k1] = np.cos(ang)
        s[k1] = np.sin(ang)
    return np.stack([c, s - c, c + s]).astype(ml_dtypes.bfloat16)


_DFT_M = _dft_consts()
LOG2E = float(np.log2(np.e))
AU = 1
IU = 8
KU = 128
BU = 16


def _cmulc(x, ang):
    c, s = float(np.cos(ang)), float(np.sin(ang))
    return (x[0] * c - x[1] * s, x[0] * s + x[1] * c)


def _cmul(x, y):
    return (x[0] * y[0] - x[1] * y[1], x[0] * y[1] + x[1] * y[0])


def _fft16_fwd(x):
    r2 = float(np.sqrt(0.5))
    c1, s1 = float(np.cos(np.pi / 8)), float(np.sin(np.pi / 8))
    Hh = [[None] * 4 for _ in range(4)]
    for a0 in range(4):
        x0, x1, x2, x3 = x[a0], x[4 + a0], x[8 + a0], x[12 + a0]
        m = x2 * r2
        t1 = (x1 * c1, x1 * s1)
        t3 = (x3 * s1, x3 * c1)
        p = x0 + m
        q = x0 - m
        u = (t1[0] + t3[0], t1[1] + t3[1])
        w = (t1[0] - t3[0], t1[1] - t3[1])
        Hh[a0][0] = (p + u[0], m + u[1])
        Hh[a0][2] = (p - u[0], m - u[1])
        Hh[a0][1] = (q + w[1], -m - w[0])
        Hh[a0][3] = (q - w[1], w[0] - m)
    G = [None] * 16
    for kp in range(4):
        t = [Hh[0][kp]] + [
            _cmulc(Hh[a0][kp], np.pi * a0 / 32 - 2 * np.pi * a0 * kp / 16) for a0 in range(1, 4)]
        s02 = (t[0][0] + t[2][0], t[0][1] + t[2][1])
        d02 = (t[0][0] - t[2][0], t[0][1] - t[2][1])
        s13 = (t[1][0] + t[3][0], t[1][1] + t[3][1])
        d13 = (t[1][0] - t[3][0], t[1][1] - t[3][1])
        G[kp] = (s02[0] + s13[0], s02[1] + s13[1])
        G[kp + 8] = (s02[0] - s13[0], s02[1] - s13[1])
        G[kp + 4] = (d02[0] + d13[1], d02[1] - d13[0])
        G[kp + 12] = (d02[0] - d13[1], d02[1] + d13[0])
    return G


def _fft16_inv(G):
    r2 = float(np.sqrt(0.5))
    c1, s1 = float(np.cos(np.pi / 8)), float(np.sin(np.pi / 8))
    J = [[None] * 4 for _ in range(4)]
    for kp in range(4):
        g0, g1, g2, g3 = G[kp], G[kp + 4], G[kp + 8], G[kp + 12]
        s02 = (g0[0] + g2[0], g0[1] + g2[1])
        d02 = (g0[0] - g2[0], g0[1] - g2[1])
        s13 = (g1[0] + g3[0], g1[1] + g3[1])
        d13 = (g1[0] - g3[0], g1[1] - g3[1])
        J[kp][0] = (s02[0] + s13[0], s02[1] + s13[1])
        J[kp][2] = (s02[0] - s13[0], s02[1] - s13[1])
        J[kp][1] = (d02[0] - d13[1], d02[1] + d13[0])
        J[kp][3] = (d02[0] + d13[1], d02[1] - d13[0])
    y = [None] * 16
    for a0 in range(4):
        t = [J[kp][a0] if (a0 == 0) else
             _cmulc(J[kp][a0], 2 * np.pi * a0 * kp / 16 - np.pi * a0 / 32) for kp in range(4)]
        s02 = (t[0][0] + t[2][0], t[0][1] + t[2][1])
        d02 = (t[0][0] - t[2][0], t[0][1] - t[2][1])
        s13 = (t[1][0] + t[3][0], t[1][1] + t[3][1])
        d13 = (t[1][0] - t[3][0], t[1][1] - t[3][1])
        z0r = s02[0] + s13[0]
        z2 = (s02[0] - s13[0], s02[1] - s13[1])
        z1 = (d02[0] - d13[1], d02[1] + d13[0])
        z3 = (d02[0] + d13[1], d02[1] - d13[0])
        y[a0] = z0r
        y[4 + a0] = z1[0] * c1 + z1[1] * s1
        y[8 + a0] = (z2[0] + z2[1]) * r2
        y[12 + a0] = z3[0] * s1 + z3[1] * c1
    return y


def _ln_t(x):
    m = jnp.mean(x, axis=0, keepdims=True)
    xc = x - m
    v = jnp.mean(xc * xc, axis=0, keepdims=True)
    return xc * lax.rsqrt(v + 1e-5)


def _phi(p):
    sl = [p[8 * f:8 * f + 8] for f in range(16)]
    mx = functools.reduce(jnp.maximum, sl)
    mn = functools.reduce(jnp.minimum, sl)
    ep = [jnp.exp2(s - mx) for s in sl]
    en = [jnp.exp2(mn - s) for s in sl]
    rp = 1.0 / functools.reduce(jnp.add, ep)
    rn = 1.0 / functools.reduce(jnp.add, en)
    out = jnp.concatenate([e * rp for e in ep] + [e * rn for e in en], axis=0)
    return out


TK = 512
TQ = 256


def _kernel(x_hbm, wqkv_hbm, wphi_ref, wo_hbm, are_ref, aim_ref, bre_ref, bim_ref, cre_ref, cim_ref,
            ldt_ref, dsk_ref, dm_hbm, o_hbm,
            xt, un, xn0, xn1, wt, wot, gb, gp, kh, tb, stp, kbuf, dcol, lhs_s, p0, p1r, pq_s, kvacc, zacc,
            xin_v, wqkv_v, wo_v, dm, ob0, ob1, ab0, ab1, dts, sems):
    i32 = jnp.int32
    cp_x = pltpu.make_async_copy(x_hbm, xin_v, sems.at[0])
    cp_w = pltpu.make_async_copy(wqkv_hbm, wqkv_v, sems.at[1])
    cp_o = pltpu.make_async_copy(wo_hbm, wo_v, sems.at[2])
    cp_d = pltpu.make_async_copy(dm_hbm, dm, sems.at[3])
    cp_w.start()
    cp_o.start()
    cp_x.start()
    cp_d.start()

    with jax.named_scope("kgen_tab"):
        dts[...] = jnp.broadcast_to(ldt_ref[...].astype(F32).reshape(1, D), (128, 512)).T
        dcol[...] = jnp.broadcast_to(dsk_ref[...].astype(F32).reshape(1, D), (128, 512)).T
        RC = 32

        def tabs(i, _):
            r0 = i * RC
            rs = slice(r0, r0 + RC)
            dt = jnp.exp(dts[rs, :]).astype(BF16).astype(F32)
            ar = dt * are_ref[rs, :].astype(F32)
            ai = dt * aim_ref[rs, :].astype(F32)
            mag = jnp.exp(ar)
            lam = (mag * jnp.cos(ai), mag * jnp.sin(ai))
            db = (dt * bre_ref[rs, :].astype(F32), dt * bim_ref[rs, :].astype(F32))
            w = _cmul((cre_ref[rs, :].astype(F32), cim_ref[rs, :].astype(F32)), db)
            l2 = _cmul(lam, lam)
            l4 = _cmul(l2, l2)
            l8 = _cmul(l4, l4)
            l16 = _cmul(l8, l8)
            stp[0, rs, :] = l16[0]
            stp[1, rs, :] = l16[1]
            stp[6, rs, :] = lam[0]
            stp[7, rs, :] = lam[1]
            p = (jnp.ones_like(ar), jnp.zeros_like(ar))
            for j in range(8):
                tb[0, pl.ds(r0 * 8 + j, RC, stride=8), :] = p[0]
                tb[1, pl.ds(r0 * 8 + j, RC, stride=8), :] = p[1]
                if j < 7:
                    p = _cmul(p, l2)
            l32 = _cmul(l16, l16)
            l64 = _cmul(l32, l32)
            l128 = _cmul(l64, l64)
            l256 = _cmul(l128, l128)
            stp[2, rs, :] = l128[0]
            stp[3, rs, :] = -l128[1]
            stp[4, rs, :] = l64[0]
            stp[5, rs, :] = -l64[1]
            stpc = (l256[0], -l256[1])
            p = (w[0], -w[1])
            for j in range(8):
                tb[2, pl.ds(r0 * 8 + j, RC, stride=8), :] = p[0]
                tb[3, pl.ds(r0 * 8 + j, RC, stride=8), :] = p[1]
                if j < 7:
                    p = _cmul(p, stpc)
            return 0
        for ii in range(D // RC):
            tabs(ii, 0)

    with jax.named_scope("kgen_mm"):
        lane = lax.broadcasted_iota(i32, (16, 128), 1)
        lo = lane < 64
        pk = lambda x0, x1: pltpu.bitcast(pltpu.pack_elementwise([x0, x1], packed_dtype=BF16), BF16)

        def kg(i, _):
            for u in range(KU):
                Bs_r, Bs_i, As_r, As_i = [], [], [], []
                for e in range(2):
                    d = (i * KU + u) * 2 + e
                    d8 = pl.multiple_of(d * 8, 8)
                    bc = lambda k: jnp.broadcast_to(stp[k, pl.ds(d, 1), :], (8, 128))
                    s16 = (bc(0), bc(1))
                    ev = (tb[0, pl.ds(d8, 8), :], tb[1, pl.ds(d8, 8), :])
                    od = _cmul(ev, (bc(6), bc(7)))
                    for _k in range(4):
                        if _k:
                            ev = _cmul(ev, s16)
                            od = _cmul(od, s16)
                        Bs_r.append(pk(ev[0], od[0]))
                        Bs_i.append(pk(ev[1], od[1]))
                    a0 = (tb[2, pl.ds(d8, 8), :], tb[3, pl.ds(d8, 8), :])
                    a1 = _cmul(a0, (bc(2), bc(3)))
                    s64 = (bc(4), bc(5))
                    a2 = _cmul(a0, s64)
                    a3 = _cmul(a1, s64)
                    As_r += [pk(a0[0], a1[0]), pk(a2[0], a3[0])]
                    As_i += [pk(a0[1], a1[1]), pk(a2[1], a3[1])]
                cat = lambda z: jnp.concatenate(z, axis=0)
                lhs = jnp.concatenate([cat(As_r), cat(As_i)], axis=1)
                rhs = jnp.concatenate([cat(Bs_r), cat(Bs_i)], axis=1)
                out = lax.dot_general(lhs, rhs, NT, preferred_element_type=F32)
                t0 = jnp.where(lo, out[0:16], pltpu.roll(out[16:32], 64, 1))
                t1 = jnp.where(lo, pltpu.roll(out[32:48], 64, 1), out[48:64])
                d0 = (i * KU + u) * 2
                kbuf[pl.ds(d0, 16, stride=512), :] = t0
                kbuf[pl.ds(d0 + 1, 16, stride=512), :] = t1
            return 0
        lax.fori_loop(0, 256 // KU, kg, 0)

    def astage(src_fn, off):
        def body(rt, _):
            for q in range(AU):
                r0 = pl.multiple_of((rt * AU + q) * 16, 16)
                G = _fft16_fwd(src_fn(r0))
                for k1 in range(16):
                    gb[k1, 0, pl.ds(r0, 16), :] = G[k1][0].astype(BF16)
                    gb[k1, 1, pl.ds(r0, 16), :] = G[k1][1].astype(BF16)
                    gb[k1, 2, pl.ds(r0, 16), :] = (G[k1][0] + G[k1][1]).astype(BF16)
            return 0
        lax.fori_loop(0, 32 // AU, body, 0)

    with jax.named_scope("kfft_a"):
        astage(lambda r0: [kbuf[pl.ds(512 * a + r0, 16), :] for a in range(16)], 0)

    with jax.named_scope("kfft_b"):
        cp_d.wait()

        def kb(i, _):
            for uu in range(BU):
                k1 = i * BU + uu
                t1 = lax.dot_general(gb[k1, 2], dm[0, k1], NN, preferred_element_type=F32)
                t2 = lax.dot_general(gb[k1, 0], dm[1, k1], NN, preferred_element_type=F32)
                t3 = lax.dot_general(gb[k1, 1], dm[2, k1], NN, preferred_element_type=F32)
                kh[k1, 0] = (t1 - t3) * (1.0 / 2048)
                kh[k1, 1] = (t1 + t2) * (1.0 / 2048)
            return 0
        lax.fori_loop(0, 16 // BU, kb, 0)

    with jax.named_scope("prep"):
        cp_w.wait()
        cp_o.wait()
        r = lax.broadcasted_iota(i32, (128, 128), 0)
        c = lax.broadcasted_iota(i32, (128, 128), 1)
        pv = jnp.where((r // 8 == c % 16) & (r % 8 == c // 16), 1.0, 0.0).astype(BF16)
        w2 = wphi_ref[...]
        re_ = lax.broadcasted_iota(i32, (32, 128), 0)
        ce_ = lax.broadcasted_iota(i32, (32, 128), 1)
        rl = lax.broadcasted_iota(i32, (128, 256), 0)
        cl = lax.broadcasted_iota(i32, (128, 256), 1)
        lmat = jnp.where(rl // 8 == cl % 16, 1.0, 0.0).astype(BF16)
        rd = lax.broadcasted_iota(i32, (256, 128), 0)
        cd = lax.broadcasted_iota(i32, (256, 128), 1)
        dmask = (rd // 16) == (cd % 16)
        hmask = (r % 8) == (c // 16)
        for g in range(4):
            eg = jnp.where(re_ == 8 * g + ce_ // 16, 1.0, 0.0).astype(BF16)
            m1_ = jnp.where(dmask, lax.dot_general(w2, eg, NN, preferred_element_type=F32), 0.0).astype(BF16)
            pg = jnp.where(hmask, lax.dot_general(lmat, m1_, NN, preferred_element_type=F32), 0.0).astype(BF16)
            for j in range(3):
                wg = wqkv_v[:, 512 * j + 128 * g:512 * j + 128 * g + 128]
                pm = pg if j < 2 else pv
                wf = lax.dot_general(pm, wg, NT, preferred_element_type=F32)
                if j < 2:
                    wf = wf * LOG2E
                wt[512 * j + 128 * g:512 * j + 128 * g + 128, :] = wf.astype(BF16)
            tmp = lax.dot_general(pv, wo_v[128 * g:128 * g + 128, :], NN, preferred_element_type=F32)
            wot[:, 128 * g:128 * g + 128] = tmp.T.astype(BF16)
    cp_x.wait()

    def attention(first):
        with jax.named_scope("a_kv"):
            NTL = S // TK

            def st0(t, xr):
                for u in range(TK // 128):
                    t0 = pl.multiple_of(t * TK + 128 * u, 128)
                    if first:
                        xv = xin_v[pl.ds(t0, 128), :].astype(F32).T
                        xt[:, pl.ds(t0, 128)] = xv
                    else:
                        xv = xt[:, pl.ds(t0, 128)]
                    xr[:, 128 * u:128 * u + 128] = _ln_t(xv).astype(BF16)

            def qkv(xr, pref):
                pref[...] = lax.dot_general(wt[...], xr[...], NN, preferred_element_type=F32)

            def soft(t, pref):
                t0 = pl.multiple_of(t * TK, TK)
                for g in range(4):
                    pq_s[256 * g:256 * g + 256, pl.ds(t0, TK)] = _phi(pref[128 * g:128 * g + 128, :]).astype(BF16)
                    phf = _phi(pref[512 + 128 * g:512 + 128 * g + 128, :])
                    v = pref[1024 + 128 * g:1024 + 128 * g + 128, :].astype(BF16)
                    kvacc[g] += lax.dot_general(phf.astype(BF16), v, NT, preferred_element_type=F32)
                    z = zacc[g]
                    for j in range(TK // 128):
                        z = z + phf[:, 128 * j:128 * j + 128]
                    zacc[g] = z
            kvacc[...] = jnp.zeros_like(kvacc)
            zacc[...] = jnp.zeros_like(zacc)
            st0(0, xn0)
            st0(1, xn1)
            qkv(xn0, p0)

            def p1(i, _):
                st0(2 * i + 2, xn0)
                qkv(xn1, p1r)
                soft(2 * i, p0)
                st0(2 * i + 3, xn1)
                qkv(xn0, p0)
                soft(2 * i + 1, p1r)
                return 0
            lax.fori_loop(0, NTL // 2 - 1, p1, 0)
            qkv(xn1, p1r)
            soft(NTL - 2, p0)
            soft(NTL - 1, p1r)
            rr = lax.broadcasted_iota(i32, (128, 256), 0)
            cc = lax.broadcasted_iota(i32, (128, 256), 1)
            m1 = (rr % 8) == (cc % 8)
            r8 = lax.broadcasted_iota(i32, (16, 256), 0)
            c8 = lax.broadcasted_iota(i32, (16, 256), 1)
            m2 = r8 == (c8 % 8)
            for g in range(4):
                lhs_s[g, 0:128, :] = jnp.where(m1, kvacc[g].T, 0.0).astype(BF16)
                zrow = jnp.sum(zacc[g].T, axis=0, keepdims=True)
                lhs_s[g, 128:144, :] = jnp.where(m2, jnp.broadcast_to(zrow, (16, 256)), 0.0).astype(BF16)
        with jax.named_scope("a_q"):
            NTL = S // TQ

            def sx(t, oref):
                t0 = pl.multiple_of(t * TQ, TQ)
                for g in range(4):
                    ph = pq_s[256 * g:256 * g + 256, pl.ds(t0, TQ)]
                    nd = lax.dot_general(lhs_s[g], ph, NN, preferred_element_type=F32)
                    rden = 1.0 / (nd[128:136] + 1e-6)
                    oref[128 * g:128 * g + 128, :] = jnp.concatenate(
                        [nd[8 * dd:8 * dd + 8] * rden for dd in range(16)], axis=0).astype(BF16)

            def sy1(t, oref, aref):
                t0 = pl.multiple_of(t * TQ, TQ)
                aref[...] = xt[:, pl.ds(t0, TQ)] + lax.dot_general(
                    wot[...], oref[...], NN, preferred_element_type=F32)

            def sy2(t, aref):
                t0 = pl.multiple_of(t * TQ, TQ)
                acc = aref[...]
                u = _ln_t(acc)
                un[:, pl.ds(t0, TQ)] = u
                dcv = dcol[...]
                xt[:, pl.ds(t0, TQ)] = acc + u * jnp.concatenate([dcv] * (TQ // 128), axis=1)
            sx(0, ob0)
            sx(1, ob1)
            sy1(0, ob0, ab0)

            def p2(i, _):
                sx(2 * i + 2, ob0)
                sy1(2 * i + 1, ob1, ab1)
                sy2(2 * i, ab0)
                sx(2 * i + 3, ob1)
                sy1(2 * i + 2, ob0, ab0)
                sy2(2 * i + 1, ab1)
                return 0
            lax.fori_loop(0, NTL // 2 - 1, p2, 0)
            sy1(NTL - 1, ob1, ab1)
            sy2(NTL - 2, ab0)
            sy2(NTL - 1, ab1)

    def conv(first):
        with jax.named_scope("b_a"):
            astage(lambda r0: [un[pl.ds(r0, 16), 128 * a:128 * a + 128] for a in range(16)], 0)
        with jax.named_scope("b_b"):
            def bb(i, _):
                for uu in range(BU):
                    k1 = i * BU + uu
                    m0, m1, m2 = dm[0, k1], dm[1, k1], dm[2, k1]
                    t1 = lax.dot_general(gb[k1, 2], m0, NN, preferred_element_type=F32)
                    t2 = lax.dot_general(gb[k1, 0], m1, NN, preferred_element_type=F32)
                    t3 = lax.dot_general(gb[k1, 1], m2, NN, preferred_element_type=F32)
                    xr, xi = t1 - t3, t1 + t2
                    kr, ki = kh[k1, 0], kh[k1, 1]
                    yr = xr * kr - xi * ki
                    yi = xr * ki + xi * kr
                    t1 = lax.dot_general((yr + yi).astype(BF16), m0, NT, preferred_element_type=F32)
                    t2 = lax.dot_general(yr.astype(BF16), m2, NT, preferred_element_type=F32)
                    t3 = lax.dot_general(yi.astype(BF16), m1, NT, preferred_element_type=F32)
                    gp[k1, 0] = t1 + t3
                    gp[k1, 1] = t1 - t2
                return 0
            lax.fori_loop(0, 16 // BU, bb, 0)
        with jax.named_scope("b_i"):
            def ocopy(g):
                return pltpu.make_async_copy(xin_v.at[:, pl.ds(g * 128, 128)], o_hbm.at[:, pl.ds(g * 128, 128)],
                                             sems.at[4 + g])
            for g in range(4):
                def body(rt, _):
                    for q in range(IU):
                        r0 = pl.multiple_of(g * 128 + (rt * IU + q) * 8, 8)
                        G = [(gp[k1, 0, pl.ds(r0, 8), :], gp[k1, 1, pl.ds(r0, 8), :]) for k1 in range(16)]
                        y = _fft16_inv(G)
                        for a in range(16):
                            xt[pl.ds(r0, 8), 128 * a:128 * a + 128] = xt[pl.ds(r0, 8), 128 * a:128 * a + 128] + y[a]
                    return 0
                lax.fori_loop(0, 16 // IU, body, 0)
                if not first:
                    for t in range(16):
                        xin_v[t * 128:t * 128 + 128, g * 128:g * 128 + 128] = (
                            xt[g * 128:g * 128 + 128, t * 128:t * 128 + 128].T.astype(BF16))
                    ocopy(g).start()
            if not first:
                for g in range(4):
                    ocopy(g).wait()

    attention(True)
    conv(True)
    attention(False)
    conv(False)

@jax.jit
def pallas_interleave_layers__linear_kernel_hedgehog__ssm_conv_s4__prompt_kernel(
    A_x, A_wqkv, A_w_phi, A_wo, B_u, B_A_re, B_A_im, B_B_re, B_B_im, B_C_re, B_C_im, B_log_dt, B_Dskip,
):
    del B_u
    vm = pl.BlockSpec(memory_space=pltpu.VMEM)
    hb = pl.BlockSpec(memory_space=pl.ANY)
    out = pl.pallas_call(
        _kernel,
        out_shape=jax.ShapeDtypeStruct((S, D), BF16),
        in_specs=[hb, hb, vm, hb, vm, vm, vm, vm, vm, vm, vm, vm, hb],
        out_specs=hb,
        scratch_shapes=[
            pltpu.VMEM((D, S), F32),
            pltpu.VMEM((D, S), F32),
            pltpu.VMEM((D, TK), BF16),
            pltpu.VMEM((D, TK), BF16),
            pltpu.VMEM((3 * D, D), BF16),
            pltpu.VMEM((D, D), BF16),
            pltpu.VMEM((16, 3, D, 128), BF16),
            pltpu.VMEM((16, 2, D, 128), F32),
            pltpu.VMEM((16, 2, D, 128), F32),
            pltpu.VMEM((4, D * 8, 128), F32),
            pltpu.VMEM((8, D, 128), F32),
            pltpu.VMEM((16 * D, 128), F32),
            pltpu.VMEM((D, 128), F32),
            pltpu.VMEM((4, 144, 256), BF16),
            pltpu.VMEM((3 * D, TK), F32),
            pltpu.VMEM((3 * D, TK), F32),
            pltpu.VMEM((2 * D, S), BF16),
            pltpu.VMEM((4, 256, 128), F32),
            pltpu.VMEM((4, 256, 128), F32),
            pltpu.VMEM((S, D), BF16),
            pltpu.VMEM((D, 3 * D), BF16),
            pltpu.VMEM((D, D), BF16),
            pltpu.VMEM((3, 16, 128, 128), BF16),
            pltpu.VMEM((D, TQ), BF16),
            pltpu.VMEM((D, TQ), BF16),
            pltpu.VMEM((D, TQ), F32),
            pltpu.VMEM((D, TQ), F32),
            pltpu.VMEM((D, 128), F32),
            pltpu.SemaphoreType.DMA((8,)),
        ],
        compiler_params=pltpu.CompilerParams(vmem_limit_bytes=120 * 1024 * 1024),
    )(A_x.reshape(S, D), A_wqkv, A_w_phi.transpose(1, 2, 0).reshape(DH * DH, H), A_wo,
      B_A_re, B_A_im, B_B_re, B_B_im, B_C_re, B_C_im,
      B_log_dt, B_Dskip, jnp.asarray(_DFT_M))
    return out.reshape(1, S, D)
```
